```python
import jax
import jax.numpy as jnp

def _softmax(x, axis=-1):
    return jax.nn.softmax(x, axis=axis)
def _gelu(x):
    return jax.nn.gelu(x, approximate=True)
def _silu(x):
    return jax.nn.silu(x)
def _sigmoid(x):
    return jax.nn.sigmoid(x)
def _layernorm(x, axis=-1, eps=1e-5):
    m = jnp.mean(x, axis=axis, keepdims=True)
    v = jnp.var(x, axis=axis, keepdims=True)
    return (x - m) / jnp.sqrt(v + eps)
def _scatter_add(tgt, idx, src, axis=0):
    return tgt.at[idx].add(src)
def _segment_sum(src, seg, n):
    return jax.ops.segment_sum(src, seg, n)
class _Rng:
    def __init__(self, key):
        self._k = key
    def _next(self):
        self._k, sub = jax.random.split(self._k)
        return sub
    def normal(self, shape):
        return jax.random.normal(self._next(), shape, dtype=jnp.bfloat16)
    def randint(self, lo, hi, shape):
        return jax.random.randint(self._next(), shape, lo, hi, dtype=jnp.int32)
    def uniform(self, shape, lo=0.0, hi=1.0):
        return jax.random.uniform(self._next(), shape, jnp.bfloat16, lo, hi)
    def permutation(self, n):
        return jax.random.permutation(self._next(), n)


kernel_name = 'interleave_layers__sliding_block_cached__dense_activation_gelu__decode'

def _fwd_setup_inputs():
    _rng = _Rng(jax.random.key(int.from_bytes(__import__("os").urandom(4), "little")))
    _w = (lambda a: (lambda t: t.astype(jnp.bfloat16) if jnp.issubdtype(t.dtype, jnp.floating) else t)(jnp.asarray(a)))
    def _A_setup():
        B, Sq, D = 2, 1, 512
        Hq, Hkv, Sk, Dh = 32, 8, 32768, 128
        assert Hq % Hkv == 0, (Hq, Hkv)
        return {
            "x": _w((lambda *s: _rng.normal(s) * 0.05)(B, Sq, D)),
            "k_cache": _w((lambda *s: _rng.normal(s) * 0.05)(B, Hkv, Sk, Dh)),
            "v_cache": _w((lambda *s: _rng.normal(s) * 0.05)(B, Hkv, Sk, Dh)),
            "wq": _w((lambda *s: _rng.normal(s) * 0.05)(D, Hq * Dh) * (D ** -0.5)),
            "wo": _w((lambda *s: _rng.normal(s) * 0.05)(Hq * Dh, D) * ((Hq * Dh) ** -0.5)),
        }
    _A_in = _A_setup()

    def _B_setup():
        B, S, D, F = 2, 1, 512, 1792
        return {
            "x": _w((lambda *s: _rng.normal(s) * 0.05)(B, S, D)),
            "w1": _w((lambda *s: _rng.normal(s) * 0.05)(D, F) * (D ** -0.5)),
            "b1": _w((lambda *s: _rng.normal(s) * 0.05)(F) * 0.01),
            "w2": _w((lambda *s: _rng.normal(s) * 0.05)(F, D) * (F ** -0.5)),
            "b2": _w((lambda *s: _rng.normal(s) * 0.05)(D) * 0.01),
        }
    _B_in = _B_setup()

    return {
        "A_x": _A_in["x"],
        "A_k_cache": _A_in["k_cache"],
        "A_v_cache": _A_in["v_cache"],
        "A_wq": _A_in["wq"],
        "A_wo": _A_in["wo"],
        "B_x": _B_in["x"],
        "B_w1": _B_in["w1"],
        "B_b1": _B_in["b1"],
        "B_w2": _B_in["w2"],
        "B_b2": _B_in["b2"],
    }

def _fwd_reference(A_x, A_k_cache, A_v_cache, A_wq, A_wo, B_x, B_w1, B_b1, B_w2, B_b2):
    def _A_ref(x, k_cache, v_cache, wq, wo):
        B, Sq, D = x.shape
        Hq, Dh = 32, 128
        Hkv, Sk = k_cache.shape[1], k_cache.shape[2]
        W = min(4096, max(256, Sk // 4))
        rep = Hq // Hkv
        q = (lambda x, *d: x.transpose(*d))((x @ wq).reshape(B, Sq, Hq, Dh), 0, 2, 1, 3)
        k = jnp.repeat(k_cache[:, :, Sk - W:, :], rep, axis=1)
        v = jnp.repeat(v_cache[:, :, Sk - W:, :], rep, axis=1)
        scores = jnp.einsum("bhqd,bhkd->bhqk", q, k) * (Dh ** -0.5)
        p = _softmax(scores, axis=-1)
        o = jnp.einsum("bhqk,bhkd->bhqd", p, v)
        return (lambda x, *d: x.transpose(*d))(o, 0, 2, 1, 3).reshape(B, Sq, Hq * Dh) @ wo

    def _B_ref(x, w1, b1, w2, b2):
        h = jnp.einsum("bsd,df->bsf", x, w1) + b1
        h = _gelu(h)
        return jnp.einsum("bsf,fd->bsd", h, w2) + b2

    x = A_x
    x = x + _A_ref(_layernorm(x, axis=-1), A_k_cache, A_v_cache, A_wq, A_wo)
    x = x + _B_ref(_layernorm(x, axis=-1), B_w1, B_b1, B_w2, B_b2)
    x = x + _A_ref(_layernorm(x, axis=-1), A_k_cache, A_v_cache, A_wq, A_wo)
    x = x + _B_ref(_layernorm(x, axis=-1), B_w1, B_b1, B_w2, B_b2)
    return x


def setup_inputs():
    _inp = _fwd_setup_inputs()
    _gk = jax.random.fold_in(jax.random.key(int.from_bytes(__import__("os").urandom(4), "little")), 2**31 - 1)
    _shapes = [[2, 1, 512]]
    _dtypes = ['bfloat16']
    _gks = jax.random.split(_gk, len(_shapes))
    _gs = [jax.random.normal(k, s, dtype=jnp.dtype(d)) * 0.05 for k, s, d in zip(_gks, _shapes, _dtypes)]
    _inp["grad_out"] = _gs[0]
    return _inp

def reference(A_x, A_k_cache, A_v_cache, A_wq, A_wo, B_w1, B_b1, B_w2, B_b2, B_x, grad_out):
    _const = dict(B_x=B_x)
    def _f(*_d):
        return _fwd_reference(**{'A_x': _d[0], 'A_k_cache': _d[1], 'A_v_cache': _d[2], 'A_wq': _d[3], 'A_wo': _d[4], 'B_w1': _d[5], 'B_b1': _d[6], 'B_w2': _d[7], 'B_b2': _d[8], **_const})
    _out, _vjp = jax.vjp(_f, A_x, A_k_cache, A_v_cache, A_wq, A_wo, B_w1, B_b1, B_w2, B_b2)
    _grads = _vjp(grad_out)
    _out0 = jnp.asarray(_out)
    return (_out0, *[jnp.asarray(_g) for _g in _grads])
```

```python
import jax
import jax.numpy as jnp
from jax import lax
import jax.experimental.pallas as pl
import jax.experimental.pallas.tpu as pltpu

_B, _D = 2, 512
_HQ, _HKV, _DH = 32, 8, 128
_REP = _HQ // _HKV
_F = 1792
_EPS = 1e-5
_SCALE = float(_DH) ** -0.5
_GELU_C = 0.7978845608028654
_GELU_A = 0.044715

_BF = jnp.bfloat16
_F32 = jnp.float32


def _dot_nn(a, b):
    return lax.dot_general(a, b, (((1,), (0,)), ((), ())), preferred_element_type=_F32)


def _dot_nt(a, b):
    return lax.dot_general(a, b, (((1,), (1,)), ((), ())), preferred_element_type=_F32)


def _dot_tn(a, b):
    return lax.dot_general(a, b, (((0,), (0,)), ((), ())), preferred_element_type=_F32)


def _rows(shape):
    return lax.broadcasted_iota(jnp.int32, shape, 0)


def _tile8(r0, r1, n):
    row = _rows((8, n))
    return jnp.where(row % 2 == 0, jnp.broadcast_to(r0, (8, n)), jnp.broadcast_to(r1, (8, n)))


def _rollsum(a):
    return (a + pltpu.roll(a, 2, 0)) + (pltpu.roll(a, 4, 0) + pltpu.roll(a, 6, 0))


def _ln_fwd(x):
    m = jnp.mean(x, axis=-1, keepdims=True)
    c = x - m
    v = jnp.mean(c * c, axis=-1, keepdims=True)
    r = lax.rsqrt(v + _EPS)
    return c * r, r


def _ln_bwd(dy, y, r):
    return r * (dy - jnp.mean(dy, axis=-1, keepdims=True) - y * jnp.mean(dy * y, axis=-1, keepdims=True))


def _gelu_and_grad(h):
    u = _GELU_C * (h + _GELU_A * h * h * h)
    t = jnp.tanh(u)
    g = 0.5 * h * (1.0 + t)
    dg = 0.5 * (1.0 + t) + 0.5 * h * (1.0 - t * t) * _GELU_C * (1.0 + 3.0 * _GELU_A * h * h)
    return g, dg


def _select4(full, h):
    row = _rows((8, _DH)) // 2
    base = h * _REP * _DH
    s = [full[:, base + r * _DH: base + (r + 1) * _DH] for r in range(_REP)]
    return jnp.where(row == 0, s[0], jnp.where(row == 1, s[1], jnp.where(row == 2, s[2], s[3])))


def _make_kernel(SK, W):
    ZR = SK - W

    def kernel(x_hbm, k_hbm, v_hbm, wq_hbm, wo_hbm, w1_hbm, b1_hbm, w2_hbm, b2_hbm, g_hbm,
               out_hbm, dx_hbm, dk_hbm, dv_hbm, dwq_hbm, dwo_hbm, dw1_hbm, db1_hbm, dw2_hbm, db2_hbm,
               kbuf, vbuf, wq, wo, w1, w2, xs, gs, b1s, b2s, zbuf,
               p_scr, ds_scr, q_scr, do_scr, t_scr, n_scr, da_scr, of_scr, dqf_scr,
               dwq_s, dwo_s, dw1_s, dw2_s, outs, dxs, db1s, db2s,
               sems):
        small = [pltpu.make_async_copy(x_hbm, xs, sems.at[0]),
                 pltpu.make_async_copy(g_hbm, gs, sems.at[0]),
                 pltpu.make_async_copy(b1_hbm, b1s, sems.at[0]),
                 pltpu.make_async_copy(b2_hbm, b2s, sems.at[0])]
        c_wq = pltpu.make_async_copy(wq_hbm, wq, sems.at[1])
        c_k = pltpu.make_async_copy(k_hbm.at[:, :, pl.ds(ZR, W), :], kbuf, sems.at[2])
        c_v = pltpu.make_async_copy(v_hbm.at[:, :, pl.ds(ZR, W), :], vbuf, sems.at[3])
        c_wo = pltpu.make_async_copy(wo_hbm, wo, sems.at[4])
        c_w1 = pltpu.make_async_copy(w1_hbm, w1, sems.at[5])
        c_w2 = pltpu.make_async_copy(w2_hbm, w2, sems.at[6])
        for c in small:
            c.start()
        c_wq.start(); c_k.start(); c_v.start(); c_wo.start(); c_w1.start(); c_w2.start()

        zbuf[...] = jnp.zeros(zbuf.shape, zbuf.dtype)

        for c in small:
            c.wait()
        c_wq.wait(); c_k.wait(); c_v.wait(); c_wo.wait(); c_w1.wait(); c_w2.wait()

        zcopies = []
        for o in (dk_hbm, dv_hbm):
            for b in range(_B):
                for h in range(_HKV):
                    c = pltpu.make_async_copy(zbuf, o.at[b, h, pl.ds(0, ZR), :], sems.at[7])
                    c.start()
                    zcopies.append(c)

        row8 = _rows((8, W))
        even8 = (row8 % 2) == 0
        even8d = (_rows((8, _DH)) % 2) == 0
        rgrp = _rows((8, _DH)) // 2

        b1v = b1s[...].reshape(1, _F).astype(_F32)
        b2v = b2s[...].reshape(1, _D).astype(_F32)

        def scatter_heads(dst, l):
            for h in range(_HKV):
                th = t_scr[h]
                for r in range(_REP):
                    c0 = (h * _REP + r) * _DH
                    dst[pl.ds(8 * l, 8), pl.ds(c0, _DH)] = jnp.where(rgrp == r, th, 0.0)

        def attn_fwd(n8, l):
            n_scr[pl.ds(8 * l, 8), :] = n8
            qall = _dot_nn(n8.astype(_BF), wq[...])
            for h in range(_HKV):
                q_scr[h, pl.ds(8 * l, 8), :] = _select4(qall, h)

            def body(h, carry):
                qh = q_scr[h, pl.ds(8 * l, 8), :].astype(_BF)
                s0 = _dot_nt(qh, kbuf[0, h])
                s1 = _dot_nt(qh, kbuf[1, h])
                s = jnp.where(even8, s0, s1) * _SCALE
                m = jnp.max(s, axis=1, keepdims=True)
                e = jnp.exp(s - m)
                p = e / jnp.sum(e, axis=1, keepdims=True)
                p_scr[h, pl.ds(8 * l, 8), :] = p
                pb = p.astype(_BF)
                o0 = _dot_nn(pb, vbuf[0, h])
                o1 = _dot_nn(pb, vbuf[1, h])
                t_scr[h] = jnp.where(even8d, o0, o1)
                return carry

            lax.fori_loop(0, _HKV, body, 0)
            scatter_heads(of_scr, l)
            a8 = _dot_nn(of_scr[pl.ds(8 * l, 8), :].astype(_BF), wo[...])
            return _rollsum(a8)

        def attn_bwd(da8, l):
            da_scr[pl.ds(8 * l, 8), :] = da8
            doall = _dot_nt(da8.astype(_BF), wo[...])
            for h in range(_HKV):
                do_scr[h, pl.ds(8 * l, 8), :] = _select4(doall, h)

            def body(h, carry):
                doh = do_scr[h, pl.ds(8 * l, 8), :].astype(_BF)
                dp0 = _dot_nt(doh, vbuf[0, h])
                dp1 = _dot_nt(doh, vbuf[1, h])
                dp = jnp.where(even8, dp0, dp1)
                p = p_scr[h, pl.ds(8 * l, 8), :]
                ds = p * (dp - jnp.sum(p * dp, axis=1, keepdims=True)) * _SCALE
                ds_scr[h, pl.ds(8 * l, 8), :] = ds
                dsb = ds.astype(_BF)
                dq0 = _dot_nn(dsb, kbuf[0, h])
                dq1 = _dot_nn(dsb, kbuf[1, h])
                t_scr[h] = jnp.where(even8d, dq0, dq1)
                return carry

            lax.fori_loop(0, _HKV, body, 0)
            scatter_heads(dqf_scr, l)
            dn8 = _dot_nt(dqf_scr[pl.ds(8 * l, 8), :].astype(_BF), wq[...])
            return _rollsum(dn8)

        def mlp_fwd(n8):
            h = _dot_nn(n8.astype(_BF), w1[...]) + b1v
            g, dg = _gelu_and_grad(h)
            m = _dot_nn(g.astype(_BF), w2[...]) + b2v
            return m, g, dg

        def mlp_bwd(dm8, dgelu):
            dg = _dot_nt(dm8.astype(_BF), w2[...])
            dh = dg * dgelu
            dn = _dot_nt(dh.astype(_BF), w1[...])
            return dn, dh

        x0 = _tile8(xs[0].astype(_F32), xs[1].astype(_F32), _D)
        n1, r1 = _ln_fwd(x0)
        x1 = x0 + attn_fwd(n1, 0)
        n2, r2 = _ln_fwd(x1)
        m2, g2, dg2 = mlp_fwd(n2)
        x2 = x1 + m2
        n3, r3 = _ln_fwd(x2)
        x3 = x2 + attn_fwd(n3, 1)
        n4, r4 = _ln_fwd(x3)
        m4, g4, dg4 = mlp_fwd(n4)
        x4 = x3 + m4
        outs[0] = x4[0:1].astype(_BF)
        outs[1] = x4[1:2].astype(_BF)
        c_out = pltpu.make_async_copy(outs, out_hbm, sems.at[8])
        c_out.start()

        dx4 = _tile8(gs[0].astype(_F32), gs[1].astype(_F32), _D)
        dn4, dh4 = mlp_bwd(dx4, dg4)
        dx3 = dx4 + _ln_bwd(dn4, n4, r4)
        dn3 = attn_bwd(dx3, 1)
        dx2 = dx3 + _ln_bwd(dn3, n3, r3)
        dn2, dh2 = mlp_bwd(dx2, dg2)
        dx1 = dx2 + _ln_bwd(dn2, n2, r2)
        dn1 = attn_bwd(dx1, 0)
        dx0 = dx1 + _ln_bwd(dn1, n1, r1)
        dxs[0] = dx0[0:1].astype(_BF)
        dxs[1] = dx0[1:2].astype(_BF)
        c_dx = pltpu.make_async_copy(dxs, dx_hbm, sems.at[9])
        c_dx.start()

        par16 = _rows((16, _DH)) % 2

        def kv_body(h, carry):
            qst = q_scr[h]
            dost = do_scr[h]
            qm = jnp.concatenate([jnp.where(par16 == 0, qst, 0.0), jnp.where(par16 == 1, qst, 0.0)],
                                 axis=1).astype(_BF)
            dom = jnp.concatenate([jnp.where(par16 == 0, dost, 0.0), jnp.where(par16 == 1, dost, 0.0)],
                                  axis=1).astype(_BF)
            dk2 = _dot_tn(ds_scr[h].astype(_BF), qm)
            kbuf[0, h] = dk2[:, :_DH].astype(_BF)
            kbuf[1, h] = dk2[:, _DH:].astype(_BF)
            dv2 = _dot_tn(p_scr[h].astype(_BF), dom)
            vbuf[0, h] = dv2[:, :_DH].astype(_BF)
            vbuf[1, h] = dv2[:, _DH:].astype(_BF)
            return carry

        lax.fori_loop(0, _HKV, kv_body, 0)
        c_dk = pltpu.make_async_copy(kbuf, dk_hbm.at[:, :, pl.ds(ZR, W), :], sems.at[2])
        c_dv = pltpu.make_async_copy(vbuf, dv_hbm.at[:, :, pl.ds(ZR, W), :], sems.at[3])
        c_dk.start(); c_dv.start()

        dwq_s[...] = _dot_tn(n_scr[...].astype(_BF), dqf_scr[...].astype(_BF)).astype(_BF)
        c_dwq = pltpu.make_async_copy(dwq_s, dwq_hbm, sems.at[1])
        c_dwq.start()
        dwo_s[...] = _dot_tn(of_scr[...].astype(_BF), da_scr[...].astype(_BF)).astype(_BF)
        c_dwo = pltpu.make_async_copy(dwo_s, dwo_hbm, sems.at[4])
        c_dwo.start()

        rF = _rows((8, _F))
        rD = _rows((8, _D))
        nst = jnp.where(rD < 2, n2, n4)
        dhst = jnp.where(rF < 2, dh2, jnp.where(rF < 4, dh4, 0.0))
        gst = jnp.where(rF < 2, g2, g4)
        dmst = jnp.where(rD < 2, dx2, jnp.where(rD < 4, dx4, 0.0))
        dw1_s[...] = _dot_tn(nst.astype(_BF), dhst.astype(_BF)).astype(_BF)
        c_dw1 = pltpu.make_async_copy(dw1_s, dw1_hbm, sems.at[5])
        c_dw1.start()
        dw2_s[...] = _dot_tn(gst.astype(_BF), dmst.astype(_BF)).astype(_BF)
        c_dw2 = pltpu.make_async_copy(dw2_s, dw2_hbm, sems.at[6])
        c_dw2.start()
        db1s[...] = jnp.sum(dhst, axis=0).astype(_BF)
        db2s[...] = jnp.sum(dmst, axis=0).astype(_BF)
        c_db1 = pltpu.make_async_copy(db1s, db1_hbm, sems.at[10])
        c_db2 = pltpu.make_async_copy(db2s, db2_hbm, sems.at[11])
        c_db1.start(); c_db2.start()

        for c in zcopies:
            c.wait()
        for c in (c_out, c_dx, c_dk, c_dv, c_dwq, c_dwo, c_dw1, c_dw2, c_db1, c_db2):
            c.wait()

    return kernel


@jax.jit
def pallas_interleave_layers__sliding_block_cached__dense_activation_gelu__decode_kernel(
    A_x: jax.Array,
    A_k_cache: jax.Array,
    A_v_cache: jax.Array,
    A_wq: jax.Array,
    A_wo: jax.Array,
    B_x: jax.Array,
    B_w1: jax.Array,
    B_b1: jax.Array,
    B_w2: jax.Array,
    B_b2: jax.Array,
    grad_out: jax.Array,
):
    del B_x
    SK = A_k_cache.shape[2]
    W = min(4096, max(256, SK // 4))
    ZR = SK - W
    any_spec = pl.BlockSpec(memory_space=pl.ANY)
    sds = jax.ShapeDtypeStruct
    out_shape = (
        sds(A_x.shape, _BF), sds(A_x.shape, _BF),
        sds(A_k_cache.shape, _BF), sds(A_v_cache.shape, _BF),
        sds(A_wq.shape, _BF), sds(A_wo.shape, _BF),
        sds(B_w1.shape, _BF), sds(B_b1.shape, _BF),
        sds(B_w2.shape, _BF), sds(B_b2.shape, _BF),
    )
    V = pltpu.VMEM
    scratch = [
        V((_B, _HKV, W, _DH), _BF),
        V((_B, _HKV, W, _DH), _BF),
        V((_D, _HQ * _DH), _BF),
        V((_HQ * _DH, _D), _BF),
        V((_D, _F), _BF),
        V((_F, _D), _BF),
        V((_B, 1, _D), _BF),
        V((_B, 1, _D), _BF),
        V((_F,), _BF),
        V((_D,), _BF),
        V((ZR, _DH), _BF),
        V((_HKV, 16, W), _F32),
        V((_HKV, 16, W), _F32),
        V((_HKV, 16, _DH), _F32),
        V((_HKV, 16, _DH), _F32),
        V((_HKV, 8, _DH), _F32),
        V((16, _D), _F32),
        V((16, _D), _F32),
        V((16, _HQ * _DH), _F32),
        V((16, _HQ * _DH), _F32),
        V((_D, _HQ * _DH), _BF),
        V((_HQ * _DH, _D), _BF),
        V((_D, _F), _BF),
        V((_F, _D), _BF),
        V((_B, 1, _D), _BF),
        V((_B, 1, _D), _BF),
        V((_F,), _BF),
        V((_D,), _BF),
        pltpu.SemaphoreType.DMA((12,)),
    ]
    return pl.pallas_call(
        _make_kernel(SK, W),
        in_specs=[any_spec] * 10,
        out_specs=tuple([any_spec] * 10),
        out_shape=out_shape,
        scratch_shapes=scratch,
        compiler_params=pltpu.CompilerParams(vmem_limit_bytes=110 * 1024 * 1024),
    )(A_x, A_k_cache, A_v_cache, A_wq, A_wo, B_w1, B_b1, B_w2, B_b2, grad_out)
```

```python
import jax
import jax.numpy as jnp
from jax import lax
import jax.experimental.pallas as pl
import jax.experimental.pallas.tpu as pltpu

_B, _D = 2, 512
_HQ, _HKV, _DH = 32, 8, 128
_REP = _HQ // _HKV
_F = 1792
_EPS = 1e-5
_SCALE = float(_DH) ** -0.5
_GELU_C = 0.7978845608028654
_GELU_A = 0.044715

_CH = 128
_WQ3 = (4, _D // 4, _HQ * _DH)
_WO3 = (4, _HQ * _DH // 4, _D)
_W13 = (2, _D // 2, _F)
_W23 = (2, _F // 2, _D)
_Z0 = 64
_ZL = 12

_BF = jnp.bfloat16
_F32 = jnp.float32


def _dot_nn(a, b):
    return lax.dot_general(a, b, (((1,), (0,)), ((), ())), preferred_element_type=_F32)


def _dot_nt(a, b):
    return lax.dot_general(a, b, (((1,), (1,)), ((), ())), preferred_element_type=_F32)


def _dot_tn(a, b):
    return lax.dot_general(a, b, (((0,), (0,)), ((), ())), preferred_element_type=_F32)


def _rows(shape):
    return lax.broadcasted_iota(jnp.int32, shape, 0)


def _tile8(r0, r1, n):
    row = _rows((8, n))
    return jnp.where(row % 2 == 0, jnp.broadcast_to(r0, (8, n)), jnp.broadcast_to(r1, (8, n)))


def _rollsum(a):
    return (a + pltpu.roll(a, 2, 0)) + (pltpu.roll(a, 4, 0) + pltpu.roll(a, 6, 0))


def _ln_fwd(x):
    m = jnp.mean(x, axis=-1, keepdims=True)
    c = x - m
    v = jnp.mean(c * c, axis=-1, keepdims=True)
    r = lax.rsqrt(v + _EPS)
    return c * r, r


def _ln_bwd(dy, y, r):
    return r * (dy - jnp.mean(dy, axis=-1, keepdims=True) - y * jnp.mean(dy * y, axis=-1, keepdims=True))


def _gelu_and_grad(h):
    u = _GELU_C * (h + _GELU_A * h * h * h)
    t = jnp.tanh(u)
    g = 0.5 * h * (1.0 + t)
    dg = 0.5 * (1.0 + t) + 0.5 * h * (1.0 - t * t) * _GELU_C * (1.0 + 3.0 * _GELU_A * h * h)
    return g, dg


def _select4(full, h):
    row = _rows((8, _DH)) // 2
    base = h * _REP * _DH
    s = [full[:, base + r * _DH: base + (r + 1) * _DH] for r in range(_REP)]
    return jnp.where(row == 0, s[0], jnp.where(row == 1, s[1], jnp.where(row == 2, s[2], s[3])))


def _make_kernel(SK, W):
    ZR = SK - W
    NC = SK // W
    n_r = W // _CH
    n_z = _B * (NC - 1) * n_r
    n_w = _B * n_r

    def kernel(x_hbm, k_hbm, v_hbm, wq_hbm, wo_hbm, w1_hbm, b1_hbm, w2_hbm, b2_hbm, g_hbm,
               out_hbm, dx_hbm, dk_hbm, dv_hbm, dwq_hbm, dwo_hbm, dw1_hbm, db1_hbm, dw2_hbm, db2_hbm,
               kbuf, vbuf, wq, wo, w1, w2, xs, gs, b1s, b2s, zbuf,
               p_scr, ds_scr, q_scr, do_scr, t_scr, n_scr, da_scr, of_scr, dqf_scr,
               dwq_s, dwo_s, dw1_s, dw2_s, outs, dxs, db1s, db2s,
               sems):
        small = [pltpu.make_async_copy(x_hbm, xs, sems.at[0]),
                 pltpu.make_async_copy(g_hbm, gs, sems.at[0]),
                 pltpu.make_async_copy(b1_hbm, b1s, sems.at[0]),
                 pltpu.make_async_copy(b2_hbm, b2s, sems.at[0])]
        c_wq = pltpu.make_async_copy(wq_hbm, wq, sems.at[1])
        c_k = pltpu.make_async_copy(k_hbm.at[:, :, pl.ds(ZR, W), :], kbuf, sems.at[2])
        c_v = pltpu.make_async_copy(v_hbm.at[:, :, pl.ds(ZR, W), :], vbuf, sems.at[3])
        c_wo = pltpu.make_async_copy(wo_hbm, wo, sems.at[4])
        c_w1 = pltpu.make_async_copy(w1_hbm, w1, sems.at[5])
        c_w2 = pltpu.make_async_copy(w2_hbm, w2, sems.at[6])
        for c in small + [c_wq, c_k, c_v, c_wo, c_w1, c_w2]:
            c.start()

        zbuf[...] = jnp.zeros(zbuf.shape, zbuf.dtype)

        for c in small + [c_wq, c_k, c_v, c_wo, c_w1]:
            c.wait()

        def zero_copy(o, idx):
            t = idx // n_r
            r = pl.multiple_of((idx - t * n_r) * _CH, _CH)
            b = t // (NC - 1)
            cc = t - b * (NC - 1)
            return pltpu.make_async_copy(zbuf, o.at[b, :, cc, pl.ds(r, _CH), :], sems.at[7])

        def z_issue(o, start, count):
            def body(j, carry):
                zero_copy(o, start + j).start()
                return carry
            lax.fori_loop(0, count, body, 0)

        z_next = [0, 0]

        def z_reserve(per_iter, iters):
            a = 0 if z_next[0] < n_z else 1
            per_iter = min(per_iter, (n_z - z_next[a]) // iters)
            base = z_next[a]
            z_next[a] += per_iter * iters
            return (dk_hbm, dv_hbm)[a], base, per_iter

        zo, zb, zn = z_reserve(_Z0, 1)
        z_issue(zo, zb, zn)
        c_w2.wait()

        even8 = (_rows((8, W)) % 2) == 0
        even8d = (_rows((8, _DH)) % 2) == 0
        rgrp = _rows((8, _DH)) // 2

        b1v = b1s[...].reshape(1, _F).astype(_F32)
        b2v = b2s[...].reshape(1, _D).astype(_F32)

        def scatter_heads(dst, l):
            for h in range(_HKV):
                th = t_scr[h]
                for r in range(_REP):
                    c0 = (h * _REP + r) * _DH
                    dst[pl.ds(8 * l, 8), pl.ds(c0, _DH)] = jnp.where(rgrp == r, th, 0.0)

        def attn_fwd(n8, l):
            n_scr[pl.ds(8 * l, 8), :] = n8
            qall = _dot_nn(n8.astype(_BF), wq[...])
            for h in range(_HKV):
                q_scr[h, pl.ds(8 * l, 8), :] = _select4(qall, h)
            zo, zb, zn = z_reserve(_ZL, _HKV)

            def body(h, carry):
                if zn:
                    z_issue(zo, zb + h * zn, zn)
                qh = q_scr[h, pl.ds(8 * l, 8), :].astype(_BF)
                s0 = _dot_nt(qh, kbuf[0, h])
                s1 = _dot_nt(qh, kbuf[1, h])
                s = jnp.where(even8, s0, s1) * _SCALE
                m = jnp.max(s, axis=1, keepdims=True)
                e = jnp.exp(s - m)
                p = e / jnp.sum(e, axis=1, keepdims=True)
                p_scr[h, pl.ds(8 * l, 8), :] = p
                pb = p.astype(_BF)
                o0 = _dot_nn(pb, vbuf[0, h])
                o1 = _dot_nn(pb, vbuf[1, h])
                t_scr[h] = jnp.where(even8d, o0, o1)
                return carry

            lax.fori_loop(0, _HKV, body, 0)
            scatter_heads(of_scr, l)
            a8 = _dot_nn(of_scr[pl.ds(8 * l, 8), :].astype(_BF), wo[...])
            return _rollsum(a8)

        def attn_bwd(da8, l):
            da_scr[pl.ds(8 * l, 8), :] = da8
            doall = _dot_nt(da8.astype(_BF), wo[...])
            for h in range(_HKV):
                do_scr[h, pl.ds(8 * l, 8), :] = _select4(doall, h)
            zo, zb, zn = z_reserve(_ZL, _HKV)

            def body(h, carry):
                if zn:
                    z_issue(zo, zb + h * zn, zn)
                doh = do_scr[h, pl.ds(8 * l, 8), :].astype(_BF)
                dp0 = _dot_nt(doh, vbuf[0, h])
                dp1 = _dot_nt(doh, vbuf[1, h])
                dp = jnp.where(even8, dp0, dp1)
                p = p_scr[h, pl.ds(8 * l, 8), :]
                ds = p * (dp - jnp.sum(p * dp, axis=1, keepdims=True)) * _SCALE
                ds_scr[h, pl.ds(8 * l, 8), :] = ds
                dsb = ds.astype(_BF)
                dq0 = _dot_nn(dsb, kbuf[0, h])
                dq1 = _dot_nn(dsb, kbuf[1, h])
                t_scr[h] = jnp.where(even8d, dq0, dq1)
                return carry

            lax.fori_loop(0, _HKV, body, 0)
            scatter_heads(dqf_scr, l)
            dn8 = _dot_nt(dqf_scr[pl.ds(8 * l, 8), :].astype(_BF), wq[...])
            return _rollsum(dn8)

        def mlp_fwd(n8):
            h = _dot_nn(n8.astype(_BF), w1[...]) + b1v
            g, dg = _gelu_and_grad(h)
            m = _dot_nn(g.astype(_BF), w2[...]) + b2v
            return m, g, dg

        def mlp_bwd(dm8, dgelu):
            dg = _dot_nt(dm8.astype(_BF), w2[...])
            dh = dg * dgelu
            dn = _dot_nt(dh.astype(_BF), w1[...])
            return dn, dh

        xf = xs[...].astype(_F32)
        x0 = _tile8(xf[0:1], xf[1:2], _D)
        n1, r1 = _ln_fwd(x0)
        x1 = x0 + attn_fwd(n1, 0)
        n2, r2 = _ln_fwd(x1)
        m2, g2, dg2 = mlp_fwd(n2)
        x2 = x1 + m2
        n3, r3 = _ln_fwd(x2)
        x3 = x2 + attn_fwd(n3, 1)
        n4, r4 = _ln_fwd(x3)
        m4, g4, dg4 = mlp_fwd(n4)
        x4 = x3 + m4
        outs[...] = x4[0:2].astype(_BF)
        c_out = pltpu.make_async_copy(outs, out_hbm, sems.at[8])
        c_out.start()

        gf = gs[...].astype(_F32)
        dx4 = _tile8(gf[0:1], gf[1:2], _D)
        dn4, dh4 = mlp_bwd(dx4, dg4)
        dx3 = dx4 + _ln_bwd(dn4, n4, r4)
        dn3 = attn_bwd(dx3, 1)
        dx2 = dx3 + _ln_bwd(dn3, n3, r3)
        dn2, dh2 = mlp_bwd(dx2, dg2)
        dx1 = dx2 + _ln_bwd(dn2, n2, r2)
        dn1 = attn_bwd(dx1, 0)
        dx0 = dx1 + _ln_bwd(dn1, n1, r1)
        dxs[...] = dx0[0:2].astype(_BF)
        c_dx = pltpu.make_async_copy(dxs, dx_hbm, sems.at[9])
        c_dx.start()

        par16 = _rows((16, _DH)) % 2
        zo, zb, zn = z_reserve(_ZL, _HKV)

        def kv_body(h, carry):
            if zn:
                z_issue(zo, zb + h * zn, zn)
            qst = q_scr[h]
            dost = do_scr[h]
            qm = jnp.concatenate([jnp.where(par16 == 0, qst, 0.0), jnp.where(par16 == 1, qst, 0.0)],
                                 axis=1).astype(_BF)
            dom = jnp.concatenate([jnp.where(par16 == 0, dost, 0.0), jnp.where(par16 == 1, dost, 0.0)],
                                  axis=1).astype(_BF)
            dk2 = _dot_tn(ds_scr[h].astype(_BF), qm)
            kbuf[0, h] = dk2[:, :_DH].astype(_BF)
            kbuf[1, h] = dk2[:, _DH:].astype(_BF)
            dv2 = _dot_tn(p_scr[h].astype(_BF), dom)
            vbuf[0, h] = dv2[:, :_DH].astype(_BF)
            vbuf[1, h] = dv2[:, _DH:].astype(_BF)
            return carry

        lax.fori_loop(0, _HKV, kv_body, 0)

        def win_copy(src, o, sem, i):
            b = i // n_r
            r = pl.multiple_of((i - b * n_r) * _CH, _CH)
            return pltpu.make_async_copy(src.at[b, :, pl.ds(r, _CH), :], o.at[b, :, NC - 1, pl.ds(r, _CH), :], sem)

        def w_issue_k(i, carry):
            win_copy(kbuf, dk_hbm, sems.at[2], i).start()
            return carry

        def w_issue_v(i, carry):
            win_copy(vbuf, dv_hbm, sems.at[3], i).start()
            return carry

        lax.fori_loop(0, n_w, w_issue_k, 0)
        lax.fori_loop(0, n_w, w_issue_v, 0)

        wcopies = []

        def wg_out(src, dst, rows, sem):
            for i in range(src.shape[1] // rows):
                c = pltpu.make_async_copy(src.at[:, pl.ds(i * rows, rows), :],
                                          dst.at[:, pl.ds(i * rows, rows), :], sem)
                c.start()
                wcopies.append(c)

        nb = n_scr[...].astype(_BF)
        dqfb = dqf_scr[...].astype(_BF)
        for i in range(_WQ3[0]):
            dwq_s[i] = _dot_tn(nb[:, i * _WQ3[1]:(i + 1) * _WQ3[1]], dqfb).astype(_BF)
        wg_out(dwq_s, dwq_hbm, 16, sems.at[1])
        ofb = of_scr[...].astype(_BF)
        dab = da_scr[...].astype(_BF)
        for i in range(_WO3[0]):
            dwo_s[i] = _dot_tn(ofb[:, i * _WO3[1]:(i + 1) * _WO3[1]], dab).astype(_BF)
        wg_out(dwo_s, dwo_hbm, 32, sems.at[4])

        rF = _rows((8, _F))
        rD = _rows((8, _D))
        nst = jnp.where(rD < 2, n2, n4).astype(_BF)
        dhst = jnp.where(rF < 2, dh2, jnp.where(rF < 4, dh4, 0.0))
        gst = jnp.where(rF < 2, g2, g4).astype(_BF)
        dmst = jnp.where(rD < 2, dx2, jnp.where(rD < 4, dx4, 0.0))
        dhb = dhst.astype(_BF)
        dmb = dmst.astype(_BF)
        for i in range(_W13[0]):
            dw1_s[i] = _dot_tn(nst[:, i * _W13[1]:(i + 1) * _W13[1]], dhb).astype(_BF)
        wg_out(dw1_s, dw1_hbm, 16, sems.at[5])
        for i in range(_W23[0]):
            dw2_s[i] = _dot_tn(gst[:, i * _W23[1]:(i + 1) * _W23[1]], dmb).astype(_BF)
        wg_out(dw2_s, dw2_hbm, 32, sems.at[6])
        db1s[...] = jnp.sum(dhst, axis=0).astype(_BF)
        db2s[...] = jnp.sum(dmst, axis=0).astype(_BF)
        c_db1 = pltpu.make_async_copy(db1s, db1_hbm, sems.at[10])
        c_db2 = pltpu.make_async_copy(db2s, db2_hbm, sems.at[11])
        c_db1.start()
        c_db2.start()

        for a, o in enumerate((dk_hbm, dv_hbm)):
            if z_next[a] < n_z:
                z_issue(o, z_next[a], n_z - z_next[a])
                z_next[a] = n_z

        def w_wait(i, carry):
            win_copy(kbuf, dk_hbm, sems.at[2], 0).wait()
            win_copy(vbuf, dv_hbm, sems.at[3], 0).wait()
            return carry

        def z_wait(i, carry):
            zero_copy(dk_hbm, 0).wait()
            zero_copy(dv_hbm, 0).wait()
            return carry

        lax.fori_loop(0, n_w, w_wait, 0)
        for c in [c_out, c_dx, c_db1, c_db2] + wcopies:
            c.wait()
        lax.fori_loop(0, n_z, z_wait, 0)

    return kernel


@jax.jit
def pallas_interleave_layers__sliding_block_cached__dense_activation_gelu__decode_kernel(
    A_x: jax.Array,
    A_k_cache: jax.Array,
    A_v_cache: jax.Array,
    A_wq: jax.Array,
    A_wo: jax.Array,
    B_x: jax.Array,
    B_w1: jax.Array,
    B_b1: jax.Array,
    B_w2: jax.Array,
    B_b2: jax.Array,
    grad_out: jax.Array,
):
    del B_x
    SK = A_k_cache.shape[2]
    W = min(4096, max(256, SK // 4))
    assert SK % W == 0 and W % _CH == 0
    NC = SK // W
    any_spec = pl.BlockSpec(memory_space=pl.ANY)
    sds = jax.ShapeDtypeStruct
    out_shape = (
        sds((_B, _D), _BF), sds((_B, _D), _BF),
        sds((_B, _HKV, NC, W, _DH), _BF), sds((_B, _HKV, NC, W, _DH), _BF),
        sds(_WQ3, _BF), sds(_WO3, _BF),
        sds(_W13, _BF), sds(B_b1.shape, _BF),
        sds(_W23, _BF), sds(B_b2.shape, _BF),
    )
    V = pltpu.VMEM
    scratch = [
        V((_B, _HKV, W, _DH), _BF),
        V((_B, _HKV, W, _DH), _BF),
        V((_D, _HQ * _DH), _BF),
        V((_HQ * _DH, _D), _BF),
        V((_D, _F), _BF),
        V((_F, _D), _BF),
        V((_B, _D), _BF),
        V((_B, _D), _BF),
        V((_F,), _BF),
        V((_D,), _BF),
        V((_HKV, _CH, _DH), _BF),
        V((_HKV, 16, W), _F32),
        V((_HKV, 16, W), _F32),
        V((_HKV, 16, _DH), _F32),
        V((_HKV, 16, _DH), _F32),
        V((_HKV, 8, _DH), _F32),
        V((16, _D), _F32),
        V((16, _D), _F32),
        V((16, _HQ * _DH), _F32),
        V((16, _HQ * _DH), _F32),
        V(_WQ3, _BF),
        V(_WO3, _BF),
        V(_W13, _BF),
        V(_W23, _BF),
        V((_B, _D), _BF),
        V((_B, _D), _BF),
        V((_F,), _BF),
        V((_D,), _BF),
        pltpu.SemaphoreType.DMA((12,)),
    ]
    res = pl.pallas_call(
        _make_kernel(SK, W),
        in_specs=[any_spec] * 10,
        out_specs=tuple([any_spec] * 10),
        out_shape=out_shape,
        scratch_shapes=scratch,
        compiler_params=pltpu.CompilerParams(vmem_limit_bytes=110 * 1024 * 1024),
    )(A_x.reshape(_B, _D), A_k_cache, A_v_cache, A_wq, A_wo, B_w1, B_b1, B_w2, B_b2, grad_out.reshape(_B, _D))
    return (res[0].reshape(A_x.shape), res[1].reshape(A_x.shape),
            res[2].reshape(A_k_cache.shape), res[3].reshape(A_v_cache.shape),
            res[4].reshape(A_wq.shape), res[5].reshape(A_wo.shape),
            res[6].reshape(B_w1.shape), res[7], res[8].reshape(B_w2.shape), res[9])
```

```python
import jax
import jax.numpy as jnp
from jax import lax
import jax.experimental.pallas as pl
import jax.experimental.pallas.tpu as pltpu

_B, _D = 2, 512
_HQ, _HKV, _DH = 32, 8, 128
_REP = _HQ // _HKV
_F = 1792
_EPS = 1e-5
_SCALE = float(_DH) ** -0.5
_GELU_C = 0.7978845608028654
_GELU_A = 0.044715

_CH = 128
_WQ3 = (4, _D // 4, _HQ * _DH)
_WO3 = (4, _HQ * _DH // 4, _D)
_W13 = (2, _D // 2, _F)
_W23 = (2, _F // 2, _D)
_OFF = 40
_Z0 = 64
_ZL = 12

_BF = jnp.bfloat16
_F32 = jnp.float32


def _dot_nn(a, b):
    return lax.dot_general(a, b, (((1,), (0,)), ((), ())), preferred_element_type=_F32)


def _dot_nt(a, b):
    return lax.dot_general(a, b, (((1,), (1,)), ((), ())), preferred_element_type=_F32)


def _dot_tn(a, b):
    return lax.dot_general(a, b, (((0,), (0,)), ((), ())), preferred_element_type=_F32)


def _rows(shape):
    return lax.broadcasted_iota(jnp.int32, shape, 0)


def _tile8(r0, r1, n):
    row = _rows((8, n))
    return jnp.where(row % 2 == 0, jnp.broadcast_to(r0, (8, n)), jnp.broadcast_to(r1, (8, n)))


def _rollsum(a):
    return (a + pltpu.roll(a, 2, 0)) + (pltpu.roll(a, 4, 0) + pltpu.roll(a, 6, 0))


def _ln_fwd(x):
    m = jnp.mean(x, axis=-1, keepdims=True)
    c = x - m
    v = jnp.mean(c * c, axis=-1, keepdims=True)
    r = lax.rsqrt(v + _EPS)
    return c * r, r


def _ln_bwd(dy, y, r):
    return r * (dy - jnp.mean(dy, axis=-1, keepdims=True) - y * jnp.mean(dy * y, axis=-1, keepdims=True))


def _gelu_and_grad(h):
    u = _GELU_C * (h + _GELU_A * h * h * h)
    t = jnp.tanh(u)
    g = 0.5 * h * (1.0 + t)
    dg = 0.5 * (1.0 + t) + 0.5 * h * (1.0 - t * t) * _GELU_C * (1.0 + 3.0 * _GELU_A * h * h)
    return g, dg


def _select4(full, h):
    row = _rows((8, _DH)) // 2
    base = h * _REP * _DH
    s = [full[:, base + r * _DH: base + (r + 1) * _DH] for r in range(_REP)]
    return jnp.where(row == 0, s[0], jnp.where(row == 1, s[1], jnp.where(row == 2, s[2], s[3])))


def _make_kernel(SK, W):
    ZR = SK - W
    n_zb = ZR // _CH - 1
    n_z = _B * n_zb
    n_wb = W // _CH - 1
    n_w = _B * n_wb

    def kernel(x_hbm, k_hbm, v_hbm, wq_hbm, wo_hbm, w1_hbm, b1_hbm, w2_hbm, b2_hbm, g_hbm,
               out_hbm, dx_hbm, dk_hbm, dv_hbm, dwq_hbm, dwo_hbm, dw1_hbm, db1_hbm, dw2_hbm, db2_hbm,
               kbuf, vbuf, wq, wo, w1, w2, xs, gs, b1s, b2s, zbuf,
               p_scr, ds_scr, q_scr, do_scr, t_scr, n_scr, da_scr, of_scr, dqf_scr,
               dwq_s, dwo_s, dw1_s, dw2_s, outs, dxs, db1s, db2s,
               sems):
        small = [pltpu.make_async_copy(x_hbm, xs, sems.at[0]),
                 pltpu.make_async_copy(g_hbm, gs, sems.at[0]),
                 pltpu.make_async_copy(b1_hbm, b1s, sems.at[0]),
                 pltpu.make_async_copy(b2_hbm, b2s, sems.at[0])]
        c_wq = pltpu.make_async_copy(wq_hbm, wq, sems.at[1])
        c_k = pltpu.make_async_copy(k_hbm.at[:, :, pl.ds(ZR, W), :], kbuf, sems.at[2])
        c_v = pltpu.make_async_copy(v_hbm.at[:, :, pl.ds(ZR, W), :], vbuf, sems.at[3])
        c_wo = pltpu.make_async_copy(wo_hbm, wo, sems.at[4])
        c_w1 = pltpu.make_async_copy(w1_hbm, w1, sems.at[5])
        c_w2 = pltpu.make_async_copy(w2_hbm, w2, sems.at[6])
        for c in small + [c_wq, c_k, c_v, c_wo, c_w1, c_w2]:
            c.start()

        zbuf[...] = jnp.zeros(zbuf.shape, zbuf.dtype)

        for c in small + [c_wq, c_k, c_v, c_wo, c_w1]:
            c.wait()

        def zero_copy(o, idx):
            off = _OFF
            b = idx // n_zb
            r = pl.multiple_of(off + (idx - b * n_zb) * _CH, 8)
            return pltpu.make_async_copy(zbuf, o.at[b, :, pl.ds(r, _CH), :], sems.at[7])

        def zero_edges(o):
            off = _OFF
            cs = []
            for b in range(_B):
                if off:
                    cs.append(pltpu.make_async_copy(zbuf.at[:, pl.ds(0, off), :], o.at[b, :, pl.ds(0, off), :], sems.at[12]))
                cs.append(pltpu.make_async_copy(zbuf.at[:, pl.ds(0, _CH - off), :],
                                                o.at[b, :, pl.ds(off + n_zb * _CH, _CH - off), :], sems.at[12]))
            return cs

        def z_issue(o, start, count):
            def body(j, carry):
                zero_copy(o, start + j).start()
                return carry
            lax.fori_loop(0, count, body, 0)

        z_next = [0, 0]

        def z_reserve(per_iter, iters):
            a = 0 if n_z - z_next[0] >= iters else 1
            per_iter = min(per_iter, (n_z - z_next[a]) // iters)
            base = z_next[a]
            z_next[a] += per_iter * iters
            return (dk_hbm, dv_hbm)[a], base, per_iter

        zo, zb, zn = z_reserve(_Z0, 1)
        z_issue(zo, zb, zn)
        c_w2.wait()

        even8 = (_rows((8, W)) % 2) == 0
        even8d = (_rows((8, _DH)) % 2) == 0
        rgrp = _rows((8, _DH)) // 2

        b1v = b1s[...].reshape(1, _F).astype(_F32)
        b2v = b2s[...].reshape(1, _D).astype(_F32)

        def scatter_heads(dst, l):
            for h in range(_HKV):
                th = t_scr[h]
                for r in range(_REP):
                    c0 = (h * _REP + r) * _DH
                    dst[pl.ds(8 * l, 8), pl.ds(c0, _DH)] = jnp.where(rgrp == r, th, 0.0)

        def attn_fwd(n8, l):
            n_scr[pl.ds(8 * l, 8), :] = n8
            qall = _dot_nn(n8.astype(_BF), wq[...])
            for h in range(_HKV):
                q_scr[h, pl.ds(8 * l, 8), :] = _select4(qall, h)
            zo, zb, zn = z_reserve(_ZL, _HKV)

            def body(h, carry):
                if zn:
                    z_issue(zo, zb + h * zn, zn)
                qh = q_scr[h, pl.ds(8 * l, 8), :].astype(_BF)
                s0 = _dot_nt(qh, kbuf[0, h])
                s1 = _dot_nt(qh, kbuf[1, h])
                s = jnp.where(even8, s0, s1) * _SCALE
                m = jnp.max(s, axis=1, keepdims=True)
                e = jnp.exp(s - m)
                p = e / jnp.sum(e, axis=1, keepdims=True)
                p_scr[h, pl.ds(8 * l, 8), :] = p
                pb = p.astype(_BF)
                o0 = _dot_nn(pb, vbuf[0, h])
                o1 = _dot_nn(pb, vbuf[1, h])
                t_scr[h] = jnp.where(even8d, o0, o1)
                return carry

            lax.fori_loop(0, _HKV, body, 0)
            scatter_heads(of_scr, l)
            a8 = _dot_nn(of_scr[pl.ds(8 * l, 8), :].astype(_BF), wo[...])
            return _rollsum(a8)

        def attn_bwd(da8, l):
            da_scr[pl.ds(8 * l, 8), :] = da8
            doall = _dot_nt(da8.astype(_BF), wo[...])
            for h in range(_HKV):
                do_scr[h, pl.ds(8 * l, 8), :] = _select4(doall, h)
            zo, zb, zn = z_reserve(_ZL, _HKV)

            def body(h, carry):
                if zn:
                    z_issue(zo, zb + h * zn, zn)
                doh = do_scr[h, pl.ds(8 * l, 8), :].astype(_BF)
                dp0 = _dot_nt(doh, vbuf[0, h])
                dp1 = _dot_nt(doh, vbuf[1, h])
                dp = jnp.where(even8, dp0, dp1)
                p = p_scr[h, pl.ds(8 * l, 8), :]
                ds = p * (dp - jnp.sum(p * dp, axis=1, keepdims=True)) * _SCALE
                ds_scr[h, pl.ds(8 * l, 8), :] = ds
                dsb = ds.astype(_BF)
                dq0 = _dot_nn(dsb, kbuf[0, h])
                dq1 = _dot_nn(dsb, kbuf[1, h])
                t_scr[h] = jnp.where(even8d, dq0, dq1)
                return carry

            lax.fori_loop(0, _HKV, body, 0)
            scatter_heads(dqf_scr, l)
            dn8 = _dot_nt(dqf_scr[pl.ds(8 * l, 8), :].astype(_BF), wq[...])
            return _rollsum(dn8)

        def mlp_fwd(n8):
            h = _dot_nn(n8.astype(_BF), w1[...]) + b1v
            g, dg = _gelu_and_grad(h)
            m = _dot_nn(g.astype(_BF), w2[...]) + b2v
            return m, g, dg

        def mlp_bwd(dm8, dgelu):
            dg = _dot_nt(dm8.astype(_BF), w2[...])
            dh = dg * dgelu
            dn = _dot_nt(dh.astype(_BF), w1[...])
            return dn, dh

        xf = xs[...].astype(_F32)
        x0 = _tile8(xf[0:1], xf[1:2], _D)
        n1, r1 = _ln_fwd(x0)
        x1 = x0 + attn_fwd(n1, 0)
        n2, r2 = _ln_fwd(x1)
        m2, g2, dg2 = mlp_fwd(n2)
        x2 = x1 + m2
        n3, r3 = _ln_fwd(x2)
        x3 = x2 + attn_fwd(n3, 1)
        n4, r4 = _ln_fwd(x3)
        m4, g4, dg4 = mlp_fwd(n4)
        x4 = x3 + m4
        outs[...] = x4[0:2].astype(_BF)
        c_out = pltpu.make_async_copy(outs, out_hbm, sems.at[8])
        c_out.start()

        gf = gs[...].astype(_F32)
        dx4 = _tile8(gf[0:1], gf[1:2], _D)
        dn4, dh4 = mlp_bwd(dx4, dg4)
        dx3 = dx4 + _ln_bwd(dn4, n4, r4)
        dn3 = attn_bwd(dx3, 1)
        dx2 = dx3 + _ln_bwd(dn3, n3, r3)
        dn2, dh2 = mlp_bwd(dx2, dg2)
        dx1 = dx2 + _ln_bwd(dn2, n2, r2)
        dn1 = attn_bwd(dx1, 0)
        dx0 = dx1 + _ln_bwd(dn1, n1, r1)
        dxs[...] = dx0[0:2].astype(_BF)
        c_dx = pltpu.make_async_copy(dxs, dx_hbm, sems.at[9])
        c_dx.start()

        par16 = _rows((16, _DH)) % 2
        zo, zb, zn = z_reserve(_ZL, _HKV)

        def kv_body(h, carry):
            if zn:
                z_issue(zo, zb + h * zn, zn)
            qst = q_scr[h]
            dost = do_scr[h]
            qm = jnp.concatenate([jnp.where(par16 == 0, qst, 0.0), jnp.where(par16 == 1, qst, 0.0)],
                                 axis=1).astype(_BF)
            dom = jnp.concatenate([jnp.where(par16 == 0, dost, 0.0), jnp.where(par16 == 1, dost, 0.0)],
                                  axis=1).astype(_BF)
            dk2 = _dot_tn(ds_scr[h].astype(_BF), qm)
            kbuf[0, h] = dk2[:, :_DH].astype(_BF)
            kbuf[1, h] = dk2[:, _DH:].astype(_BF)
            dv2 = _dot_tn(p_scr[h].astype(_BF), dom)
            vbuf[0, h] = dv2[:, :_DH].astype(_BF)
            vbuf[1, h] = dv2[:, _DH:].astype(_BF)
            return carry

        lax.fori_loop(0, _HKV, kv_body, 0)

        def win_copy(src, o, sem, i):
            off = _OFF
            b = i // n_wb
            r = pl.multiple_of(off + (i - b * n_wb) * _CH, 8)
            return pltpu.make_async_copy(src.at[b, :, pl.ds(r, _CH), :], o.at[b, :, pl.ds(ZR + r, _CH), :], sem)

        def win_edges(src, o):
            off = _OFF
            cs = []
            for b in range(_B):
                if off:
                    cs.append(pltpu.make_async_copy(src.at[b, :, pl.ds(0, off), :], o.at[b, :, pl.ds(ZR, off), :], sems.at[13]))
                t0 = off + n_wb * _CH
                cs.append(pltpu.make_async_copy(src.at[b, :, pl.ds(t0, _CH - off), :],
                                                o.at[b, :, pl.ds(ZR + t0, _CH - off), :], sems.at[13]))
            return cs

        edges = zero_edges(dk_hbm) + zero_edges(dv_hbm) + win_edges(kbuf, dk_hbm) + win_edges(vbuf, dv_hbm)
        for c in edges:
            c.start()

        def w_issue_k(i, carry):
            win_copy(kbuf, dk_hbm, sems.at[2], i).start()
            return carry

        def w_issue_v(i, carry):
            win_copy(vbuf, dv_hbm, sems.at[3], i).start()
            return carry

        lax.fori_loop(0, n_w, w_issue_k, 0)
        lax.fori_loop(0, n_w, w_issue_v, 0)

        wcopies = []

        def wg_out(src, dst, rows, sem, csplit=1):
            cw = src.shape[2] // csplit
            for i in range(src.shape[1] // rows):
                for cc in range(csplit):
                    c = pltpu.make_async_copy(src.at[:, pl.ds(i * rows, rows), pl.ds(cc * cw, cw)],
                                              dst.at[:, pl.ds(i * rows, rows), pl.ds(cc * cw, cw)], sem)
                    c.start()
                    wcopies.append(c)

        nb = n_scr[...].astype(_BF)
        dqfb = dqf_scr[...].astype(_BF)
        for i in range(_WQ3[0]):
            dwq_s[i] = _dot_tn(nb[:, i * _WQ3[1]:(i + 1) * _WQ3[1]], dqfb).astype(_BF)
        wg_out(dwq_s, dwq_hbm, 8, sems.at[1], 2)
        ofb = of_scr[...].astype(_BF)
        dab = da_scr[...].astype(_BF)
        for i in range(_WO3[0]):
            dwo_s[i] = _dot_tn(ofb[:, i * _WO3[1]:(i + 1) * _WO3[1]], dab).astype(_BF)
        wg_out(dwo_s, dwo_hbm, 32, sems.at[4])

        rF = _rows((8, _F))
        rD = _rows((8, _D))
        nst = jnp.where(rD < 2, n2, n4).astype(_BF)
        dhst = jnp.where(rF < 2, dh2, jnp.where(rF < 4, dh4, 0.0))
        gst = jnp.where(rF < 2, g2, g4).astype(_BF)
        dmst = jnp.where(rD < 2, dx2, jnp.where(rD < 4, dx4, 0.0))
        dhb = dhst.astype(_BF)
        dmb = dmst.astype(_BF)
        for i in range(_W13[0]):
            dw1_s[i] = _dot_tn(nst[:, i * _W13[1]:(i + 1) * _W13[1]], dhb).astype(_BF)
        wg_out(dw1_s, dw1_hbm, 16, sems.at[5])
        for i in range(_W23[0]):
            dw2_s[i] = _dot_tn(gst[:, i * _W23[1]:(i + 1) * _W23[1]], dmb).astype(_BF)
        wg_out(dw2_s, dw2_hbm, 32, sems.at[6])
        db1s[...] = jnp.sum(dhst, axis=0).astype(_BF)
        db2s[...] = jnp.sum(dmst, axis=0).astype(_BF)
        c_db1 = pltpu.make_async_copy(db1s, db1_hbm, sems.at[10])
        c_db2 = pltpu.make_async_copy(db2s, db2_hbm, sems.at[11])
        c_db1.start()
        c_db2.start()

        for a, o in enumerate((dk_hbm, dv_hbm)):
            if z_next[a] < n_z:
                z_issue(o, z_next[a], n_z - z_next[a])
                z_next[a] = n_z

        def w_wait(i, carry):
            win_copy(kbuf, dk_hbm, sems.at[2], 0).wait()
            win_copy(vbuf, dv_hbm, sems.at[3], 0).wait()
            return carry

        def z_wait(i, carry):
            zero_copy(dk_hbm, 0).wait()
            zero_copy(dv_hbm, 0).wait()
            return carry

        lax.fori_loop(0, n_w, w_wait, 0)
        for c in [c_out, c_dx, c_db1, c_db2] + wcopies + edges:
            c.wait()
        lax.fori_loop(0, n_z, z_wait, 0)

    return kernel


@jax.jit
def pallas_interleave_layers__sliding_block_cached__dense_activation_gelu__decode_kernel(
    A_x: jax.Array,
    A_k_cache: jax.Array,
    A_v_cache: jax.Array,
    A_wq: jax.Array,
    A_wo: jax.Array,
    B_x: jax.Array,
    B_w1: jax.Array,
    B_b1: jax.Array,
    B_w2: jax.Array,
    B_b2: jax.Array,
    grad_out: jax.Array,
):
    del B_x
    SK = A_k_cache.shape[2]
    W = min(4096, max(256, SK // 4))
    assert (SK - W) % _CH == 0 and W % _CH == 0 and SK - W >= 2 * _CH and W >= 2 * _CH
    any_spec = pl.BlockSpec(memory_space=pl.ANY)
    sds = jax.ShapeDtypeStruct
    out_shape = (
        sds((_B, _D), _BF), sds((_B, _D), _BF),
        sds(A_k_cache.shape, _BF), sds(A_v_cache.shape, _BF),
        sds(_WQ3, _BF), sds(_WO3, _BF),
        sds(_W13, _BF), sds(B_b1.shape, _BF),
        sds(_W23, _BF), sds(B_b2.shape, _BF),
    )
    V = pltpu.VMEM
    scratch = [
        V((_B, _HKV, W, _DH), _BF),
        V((_B, _HKV, W, _DH), _BF),
        V((_D, _HQ * _DH), _BF),
        V((_HQ * _DH, _D), _BF),
        V((_D, _F), _BF),
        V((_F, _D), _BF),
        V((_B, _D), _BF),
        V((_B, _D), _BF),
        V((_F,), _BF),
        V((_D,), _BF),
        V((_HKV, _CH, _DH), _BF),
        V((_HKV, 16, W), _F32),
        V((_HKV, 16, W), _F32),
        V((_HKV, 16, _DH), _F32),
        V((_HKV, 16, _DH), _F32),
        V((_HKV, 8, _DH), _F32),
        V((16, _D), _F32),
        V((16, _D), _F32),
        V((16, _HQ * _DH), _F32),
        V((16, _HQ * _DH), _F32),
        V(_WQ3, _BF),
        V(_WO3, _BF),
        V(_W13, _BF),
        V(_W23, _BF),
        V((_B, _D), _BF),
        V((_B, _D), _BF),
        V((_F,), _BF),
        V((_D,), _BF),
        pltpu.SemaphoreType.DMA((14,)),
    ]
    res = pl.pallas_call(
        _make_kernel(SK, W),
        in_specs=[any_spec] * 10,
        out_specs=tuple([any_spec] * 10),
        out_shape=out_shape,
        scratch_shapes=scratch,
        compiler_params=pltpu.CompilerParams(vmem_limit_bytes=110 * 1024 * 1024),
    )(A_x.reshape(_B, _D), A_k_cache, A_v_cache, A_wq, A_wo, B_w1, B_b1, B_w2, B_b2, grad_out.reshape(_B, _D))
    return (res[0].reshape(A_x.shape), res[1].reshape(A_x.shape),
            res[2], res[3],
            res[4].reshape(A_wq.shape), res[5].reshape(A_wo.shape),
            res[6].reshape(B_w1.shape), res[7], res[8].reshape(B_w2.shape), res[9])
```
